```python
import jax
import jax.numpy as jnp

def _softmax(x, axis=-1):
    return jax.nn.softmax(x, axis=axis)

def _gelu(x):
    return jax.nn.gelu(x, approximate=True)

def _silu(x):
    return jax.nn.silu(x)

def _sigmoid(x):
    return jax.nn.sigmoid(x)

def _layernorm(x, axis=-1, eps=1e-05):
    m = jnp.mean(x, axis=axis, keepdims=True)
    v = jnp.var(x, axis=axis, keepdims=True)
    return (x - m) / jnp.sqrt(v + eps)

def _scatter_add(tgt, idx, src, axis=0):
    return tgt.at[idx].add(src)

def _segment_sum(src, seg, n):
    return jax.ops.segment_sum(src, seg, n)

class _Rng:

    def __init__(self, key):
        self._k = key

    def _next(self):
        self._k, sub = jax.random.split(self._k)
        return sub

    def normal(self, shape):
        return jax.random.normal(self._next(), shape, dtype=jnp.bfloat16)

    def randint(self, lo, hi, shape):
        return jax.random.randint(self._next(), shape, lo, hi, dtype=jnp.int32)

    def uniform(self, shape, lo=0.0, hi=1.0):
        return jax.random.uniform(self._next(), shape, jnp.bfloat16, lo, hi)

    def permutation(self, n):
        return jax.random.permutation(self._next(), n)
kernel_name = 'adaLN_cond__mha_block_cached__moe_arch_mod__decode'

def setup_inputs():
    _rng = _Rng(jax.random.key(int.from_bytes(__import__("os").urandom(4), "little")))
    _w = lambda a: (lambda t: t.astype(jnp.bfloat16) if jnp.issubdtype(t.dtype, jnp.floating) else t)(jnp.asarray(a))

    def _A_setup():
        B, Sq, D = (4, 1, 448)
        H, Sk, Dh = (16, 16384, 256)
        return {'x': _w((lambda *s: _rng.normal(s) * 0.05)(B, Sq, D)), 'k_cache': _w((lambda *s: _rng.normal(s) * 0.05)(B, H, Sk, Dh)), 'v_cache': _w((lambda *s: _rng.normal(s) * 0.05)(B, H, Sk, Dh)), 'wq': _w((lambda *s: _rng.normal(s) * 0.05)(D, H * Dh) * D ** (-0.5)), 'wo': _w((lambda *s: _rng.normal(s) * 0.05)(H * Dh, D) * (H * Dh) ** (-0.5))}
    _A_in = _A_setup()

    def _B_setup():
        B, S, D, F, C = (4, 1, 448, 1792, 1)
        return {'x': _w((lambda *s: _rng.normal(s) * 0.05)(B, S, D)), 'w_r': _w((lambda *s: _rng.normal(s) * 0.05)(D)), 'w_gate': _w((lambda *s: _rng.normal(s) * 0.05)(D, F)), 'w_up': _w((lambda *s: _rng.normal(s) * 0.05)(D, F)), 'w_down': _w((lambda *s: _rng.normal(s) * 0.05)(F, D))}
    _B_in = _B_setup()
    return {'A_x': _A_in['x'], 'A_k_cache': _A_in['k_cache'], 'A_v_cache': _A_in['v_cache'], 'A_wq': _A_in['wq'], 'A_wo': _A_in['wo'], 'B_x': _B_in['x'], 'B_w_r': _B_in['w_r'], 'B_w_gate': _B_in['w_gate'], 'B_w_up': _B_in['w_up'], 'B_w_down': _B_in['w_down'], 'c': _w((lambda *s: _rng.normal(s) * 0.05)(4, 448)), 'w_mod': _w((lambda *s: _rng.normal(s) * 0.05)(448, 6 * 448) * 448 ** (-0.5))}

def reference(A_x, A_k_cache, A_v_cache, A_wq, A_wo, B_x, B_w_r, B_w_gate, B_w_up, B_w_down, c, w_mod):

    def _A_ref(x, k_cache, v_cache, wq, wo):
        B, Sq, D = x.shape
        H, Dh = (16, 256)
        q = (lambda x, *d: x.transpose(*d))((x @ wq).reshape(B, Sq, H, Dh), 0, 2, 1, 3)
        scores = jnp.einsum('bhqd,bhkd->bhqk', q, k_cache) * Dh ** (-0.5)
        p = _softmax(scores, axis=-1)
        o = jnp.einsum('bhqk,bhkd->bhqd', p, v_cache)
        return (lambda x, *d: x.transpose(*d))(o, 0, 2, 1, 3).reshape(B, Sq, H * Dh) @ wo

    def _B_ref(x, w_r, w_gate, w_up, w_down):
        B, S, D = x.shape
        C = 1
        r = x @ w_r
        idx = jnp.argsort(-r, axis=-1)[:, :C]
        idx_e = jnp.repeat(idx.reshape(B, C, 1), D, axis=2)
        x_sel = jnp.take_along_axis(x, idx_e, axis=1)
        g = _silu(x_sel @ w_gate)
        u = x_sel @ w_up
        y = g * u @ w_down
        r_sel = _sigmoid(jnp.take_along_axis(r, idx, axis=1))
        y = y * r_sel.reshape(B, C, 1)
        b_off = (jnp.arange(B) * S).reshape(B, 1)
        flat_idx = (idx + b_off).reshape(B * C)
        zero = (x * 0.0).reshape(B * S, D)
        upd = _scatter_add(zero, flat_idx, y.reshape(B * C, D), axis=0)
        return x + upd.reshape(B, S, D)
    x = A_x
    mod = (_silu(c) @ w_mod).reshape(c.shape[0], 6, 1, -1)
    sa, ca, ga, sb, cb, gb = (mod[:, 0].copy(), mod[:, 1].copy(), mod[:, 2].copy(), mod[:, 3].copy(), mod[:, 4].copy(), mod[:, 5].copy())
    h = _layernorm(x, axis=-1) * (1 + ca) + sa
    x = x + ga * _A_ref(h, A_k_cache, A_v_cache, A_wq, A_wo)
    h = _layernorm(x, axis=-1) * (1 + cb) + sb
    x = x + gb * _B_ref(h, B_w_r, B_w_gate, B_w_up, B_w_down)
    return x
```

```python
import functools
import jax, jax.numpy as jnp, numpy as np
from jax import lax
from jax.experimental import pallas as pl
from jax.experimental.pallas import tpu as pltpu

B, H, SK, DH, D, F = 4, 16, 16384, 256, 448, 1792
R = 8
bf16, f32 = jnp.bfloat16, jnp.float32
NT = (((1,), (1,)), ((), ()))

def _ln(x):
    m = jnp.mean(x, axis=-1, keepdims=True)
    d = x - m
    v = jnp.mean(d * d, axis=-1, keepdims=True)
    return d / jnp.sqrt(v + 1e-5)

def _pad(a):
    return jnp.concatenate([a, jnp.zeros((R - B, a.shape[1]), a.dtype)], axis=0)

def make(T=1024, NBUF=4, SUB=64, mode="inter", WSUB=16, wlate=0):
    NC = SK // T
    N = B * H * NC
    NS = T // SUB
    def kern(x_hbm, k_hbm, v_hbm, wq_hbm, woT_hbm, wr_hbm, wg_hbm, wu_hbm, wdT_hbm, c_hbm, wmod_hbm,
             o_hbm, kbuf, vbuf, ksem, vsem, wq_v, woT_v, wg_v, wu_v, wdT_v, wmod_v, x_v, c_v, wr_v, o_v, wsem, q_scr):
        def start(i, slot):
            h = i // (B * NC)
            b = (i // NC) % B
            c = i % NC
            kc = lambda r, n, p: pltpu.make_async_copy(k_hbm.at[b, h, pl.ds(c*T + r, n), :], kbuf.at[slot, pl.ds(r, n)], ksem.at[slot]).start(priority=p)
            vc = lambda r, n, p: pltpu.make_async_copy(v_hbm.at[b, h, pl.ds(c*T + r, n), :], vbuf.at[slot, pl.ds(r, n)], vsem.at[slot]).start(priority=p)
            if mode == "inter":
                for s in range(NS):
                    kc(s*SUB, SUB, 0); vc(s*SUB, SUB, 1)
            elif mode == "halves":
                for f in (kc, vc):
                    for s in range(NS // 2):
                        f(s*SUB, SUB, 0); f(T//2 + s*SUB, SUB, 1)
            elif mode == "mixed":
                for r in range(0, T, 128):
                    kc(r, 32, 0); vc(r, 96, 1); kc(r+32, 96, 0); vc(r+96, 32, 1)
        def wcopy(src, dst, sem):
            n = src.shape[0]
            nsub = n // WSUB
            for s in range(nsub // 2):
                pltpu.make_async_copy(src.at[pl.ds(s*WSUB, WSUB)], dst.at[pl.ds(s*WSUB, WSUB)], sem).start(priority=0)
                pltpu.make_async_copy(src.at[pl.ds((s + nsub//2)*WSUB, WSUB)], dst.at[pl.ds((s + nsub//2)*WSUB, WSUB)], sem).start(priority=1)
        def wwait(dst, sem):
            pltpu.make_async_copy(dst, dst, sem).wait()
        small = [pltpu.make_async_copy(c_hbm, c_v, wsem.at[6]), pltpu.make_async_copy(x_hbm, x_v, wsem.at[7]),
                 pltpu.make_async_copy(wr_hbm, wr_v, wsem.at[8])]
        small[0].start(priority=0); small[1].start(priority=1); small[2].start(priority=1)
        wcopy(wmod_hbm, wmod_v, wsem.at[0])
        wcopy(wq_hbm, wq_v, wsem.at[1])
        for j in range(NBUF):
            start(j, j)
        wcopy(woT_hbm, woT_v, wsem.at[2])
        def late():
            wcopy(wg_hbm, wg_v, wsem.at[3])
            wcopy(wu_hbm, wu_v, wsem.at[4])
            wcopy(wdT_hbm, wdT_v, wsem.at[5])
        if not wlate: late()

        for s in small: s.wait()
        x = _pad(x_v[...].astype(f32))
        cc = _pad(c_v[...].astype(f32))
        sc = (cc * jax.nn.sigmoid(cc)).astype(bf16)
        wwait(wmod_v, wsem.at[0])
        mod = jnp.dot(sc, wmod_v[...], preferred_element_type=f32)
        sa, ca, ga, sb, cb, gb = [mod[:, i*D:(i+1)*D] for i in range(6)]
        h1 = (_ln(x) * (1 + ca) + sa).astype(bf16)
        wwait(wq_v, wsem.at[1])
        q = jnp.dot(h1, wq_v[...], preferred_element_type=f32) * (DH ** -0.5)
        for hh in range(H):
            q_scr[hh] = q[:, hh*DH:(hh+1)*DH].astype(bf16)
        wwait(woT_v, wsem.at[2])

        rowd = lax.broadcasted_iota(jnp.int32, (R, DH), 0)

        def head_body(h, y):
            qh = q_scr[h]
            def batch_body(b, oh):
                def chunk_body(c, carry):
                    m, l, acc = carry
                    i = (h * B + b) * NC + c
                    slot = i % NBUF
                    wwait(kbuf.at[slot], ksem.at[slot])
                    s = lax.dot_general(qh, kbuf[slot], NT, preferred_element_type=f32)
                    m_new = jnp.maximum(m, jnp.max(s, axis=-1, keepdims=True))
                    alpha = jnp.exp(m - m_new)
                    p = jnp.exp(s - m_new)
                    ps = p[:, 0:128]
                    for t in range(1, T // 128):
                        ps = ps + p[:, t*128:(t+1)*128]
                    l = alpha * l + ps
                    wwait(vbuf.at[slot], vsem.at[slot])
                    acc = alpha * acc + jnp.dot(p.astype(bf16), vbuf[slot], preferred_element_type=f32)
                    @pl.when(i + NBUF < N)
                    def _():
                        start(i + NBUF, slot)
                    return m_new, l, acc
                m, l, acc = lax.fori_loop(0, NC, chunk_body,
                    (jnp.full((R, 1), -jnp.inf, f32), jnp.zeros((R, 128), f32), jnp.zeros((R, DH), f32)))
                o = acc / jnp.sum(l, axis=-1, keepdims=True)
                return jnp.where(rowd == b, o, oh)
            oh = lax.fori_loop(0, B, batch_body, jnp.zeros((R, DH), f32))
            if wlate:
                @pl.when(h == wlate)
                def _(): late()
            return y + lax.dot_general(oh.astype(bf16), woT_v[:, pl.ds(pl.multiple_of(h * DH, DH), DH)], NT, preferred_element_type=f32)
        y = lax.fori_loop(0, H, head_body, jnp.zeros((R, D), f32))

        x1 = x + ga * y
        h2 = (_ln(x1) * (1 + cb) + sb).astype(bf16)
        h2f = h2.astype(f32)
        wr = wr_v[...].astype(f32).reshape(1, D)
        r = jnp.sum(h2f * wr, axis=-1, keepdims=True)
        wwait(wg_v, wsem.at[3]); wwait(wu_v, wsem.at[4]); wwait(wdT_v, wsem.at[5])
        g = jnp.dot(h2, wg_v[...], preferred_element_type=f32)
        u = jnp.dot(h2, wu_v[...], preferred_element_type=f32)
        a = (g * jax.nn.sigmoid(g) * u).astype(bf16)
        ym = lax.dot_general(a, wdT_v[...], NT, preferred_element_type=f32) * jax.nn.sigmoid(r)
        res = (x1 + gb * (h2f + (h2f * 0.0 + ym))).astype(bf16)
        o_v[...] = res[0:B]
        cp = pltpu.make_async_copy(o_v, o_hbm, wsem.at[9])
        cp.start(); cp.wait()

    def fn(A_x, A_k_cache, A_v_cache, A_wq, A_wo, B_x, B_w_r, B_w_gate, B_w_up, B_w_down, c, w_mod):
        hb = pl.BlockSpec(memory_space=pltpu.HBM)
        out = pl.pallas_call(kern,
            out_shape=jax.ShapeDtypeStruct((B, D), bf16),
            in_specs=[hb] * 11,
            out_specs=hb,
            scratch_shapes=[pltpu.VMEM((NBUF, T, DH), bf16), pltpu.VMEM((NBUF, T, DH), bf16),
                            pltpu.SemaphoreType.DMA((NBUF,)), pltpu.SemaphoreType.DMA((NBUF,)),
                            pltpu.VMEM((D, H*DH), bf16), pltpu.VMEM((D, H*DH), bf16),
                            pltpu.VMEM((D, F), bf16), pltpu.VMEM((D, F), bf16), pltpu.VMEM((D, F), bf16),
                            pltpu.VMEM((D, 6*D), bf16), pltpu.VMEM((B, D), bf16), pltpu.VMEM((B, D), bf16),
                            pltpu.VMEM((D,), bf16), pltpu.VMEM((B, D), bf16), pltpu.SemaphoreType.DMA((10,)),
                            pltpu.VMEM((H, R, DH), bf16)],
            compiler_params=pltpu.CompilerParams(vmem_limit_bytes=100*1024*1024),
        )(A_x.reshape(B, D), A_k_cache, A_v_cache, A_wq, A_wo.T, B_w_r, B_w_gate, B_w_up, B_w_down.T, c, w_mod)
        return out.reshape(B, 1, D)
    return fn


_fn = make(T=1024, NBUF=4, SUB=64)


@jax.jit
def pallas_adaLN_cond__mha_block_cached__moe_arch_mod__decode_kernel(
    A_x, A_k_cache, A_v_cache, A_wq, A_wo, B_x, B_w_r, B_w_gate, B_w_up, B_w_down, c, w_mod
):
    return _fn(A_x, A_k_cache, A_v_cache, A_wq, A_wo, B_x, B_w_r, B_w_gate, B_w_up, B_w_down, c, w_mod)
```

```python
import functools
import jax, jax.numpy as jnp, numpy as np
from jax import lax
from jax.experimental import pallas as pl
from jax.experimental.pallas import tpu as pltpu

B, H, SK, DH, D, F = 4, 16, 16384, 256, 448, 1792
R = 8
bf16, f32 = jnp.bfloat16, jnp.float32
NT = (((1,), (1,)), ((), ()))

def _ln(x):
    m = jnp.mean(x, axis=-1, keepdims=True)
    d = x - m
    v = jnp.mean(d * d, axis=-1, keepdims=True)
    return d / jnp.sqrt(v + 1e-5)

def _pad(a):
    return jnp.concatenate([a, jnp.zeros((R - B, a.shape[1]), a.dtype)], axis=0)

def make(T=1024, NBUF=4, SUB=64, mode="inter", WSUB=16, wlate=0):
    NC = SK // T
    N = B * H * NC
    NS = T // SUB
    def kern(x_hbm, k_hbm, v_hbm, wq_hbm, woT_hbm, wr_hbm, wg_hbm, wu_hbm, wdT_hbm, c_hbm, wmod_hbm,
             o_hbm, kbuf, vbuf, ksem, vsem, wq_v, woT_v, wg_v, wu_v, wdT_v, wmod_v, x_v, c_v, wr_v, o_v, wsem, q_scr):
        def start(i, slot):
            h = i // (B * NC)
            b = (i // NC) % B
            c = i % NC
            kc = lambda r, n, p: pltpu.make_async_copy(k_hbm.at[b, h, pl.ds(c*T + r, n), :], kbuf.at[slot, pl.ds(r, n)], ksem.at[slot]).start(priority=p)
            vc = lambda r, n, p: pltpu.make_async_copy(v_hbm.at[b, h, pl.ds(c*T + r, n), :], vbuf.at[slot, pl.ds(r, n)], vsem.at[slot]).start(priority=p)
            if mode == "inter":
                for r in range(0, T, SUB):
                    n = min(SUB, T - r)
                    kc(r, n, 0); vc(r, n, 1)
            elif mode == "halves":
                for f in (kc, vc):
                    for s in range(NS // 2):
                        f(s*SUB, SUB, 0); f(T//2 + s*SUB, SUB, 1)
            elif mode == "mixed":
                for r in range(0, T, 128):
                    kc(r, 32, 0); vc(r, 96, 1); kc(r+32, 96, 0); vc(r+96, 32, 1)
        def wcopy(src, dst, sem):
            n = src.shape[0]
            nsub = n // WSUB
            for s in range(nsub // 2):
                pltpu.make_async_copy(src.at[pl.ds(s*WSUB, WSUB)], dst.at[pl.ds(s*WSUB, WSUB)], sem).start(priority=0)
                pltpu.make_async_copy(src.at[pl.ds((s + nsub//2)*WSUB, WSUB)], dst.at[pl.ds((s + nsub//2)*WSUB, WSUB)], sem).start(priority=1)
        def wwait(dst, sem):
            pltpu.make_async_copy(dst, dst, sem).wait()
        small = [pltpu.make_async_copy(c_hbm, c_v, wsem.at[6]), pltpu.make_async_copy(x_hbm, x_v, wsem.at[7]),
                 pltpu.make_async_copy(wr_hbm, wr_v, wsem.at[8])]
        small[0].start(priority=0); small[1].start(priority=1); small[2].start(priority=1)
        wcopy(wmod_hbm, wmod_v, wsem.at[0])
        wcopy(wq_hbm, wq_v, wsem.at[1])
        for j in range(NBUF):
            start(j, j)
        wcopy(woT_hbm, woT_v, wsem.at[2])
        def late():
            wcopy(wg_hbm, wg_v, wsem.at[3])
            wcopy(wu_hbm, wu_v, wsem.at[4])
            wcopy(wdT_hbm, wdT_v, wsem.at[5])
        if not wlate: late()

        for s in small: s.wait()
        x = _pad(x_v[...].astype(f32))
        cc = _pad(c_v[...].astype(f32))
        sc = (cc * jax.nn.sigmoid(cc)).astype(bf16)
        wwait(wmod_v, wsem.at[0])
        mod = jnp.dot(sc, wmod_v[...], preferred_element_type=f32)
        sa, ca, ga, sb, cb, gb = [mod[:, i*D:(i+1)*D] for i in range(6)]
        h1 = (_ln(x) * (1 + ca) + sa).astype(bf16)
        wwait(wq_v, wsem.at[1])
        q = jnp.dot(h1, wq_v[...], preferred_element_type=f32) * (DH ** -0.5)
        for hh in range(H):
            q_scr[hh] = q[:, hh*DH:(hh+1)*DH].astype(bf16)
        wwait(woT_v, wsem.at[2])

        rowd = lax.broadcasted_iota(jnp.int32, (R, DH), 0)

        def head_body(h, y):
            qh = q_scr[h]
            def batch_body(b, oh):
                def chunk_body(c, carry):
                    m, l, acc = carry
                    i = (h * B + b) * NC + c
                    slot = i % NBUF
                    wwait(kbuf.at[slot], ksem.at[slot])
                    s = lax.dot_general(qh, kbuf[slot], NT, preferred_element_type=f32)
                    m_new = jnp.maximum(m, jnp.max(s, axis=-1, keepdims=True))
                    alpha = jnp.exp(m - m_new)
                    p = jnp.exp(s - m_new)
                    ps = p[:, 0:128]
                    for t in range(1, T // 128):
                        ps = ps + p[:, t*128:(t+1)*128]
                    l = alpha * l + ps
                    wwait(vbuf.at[slot], vsem.at[slot])
                    acc = alpha * acc + jnp.dot(p.astype(bf16), vbuf[slot], preferred_element_type=f32)
                    @pl.when(i + NBUF < N)
                    def _():
                        start(i + NBUF, slot)
                    return m_new, l, acc
                m, l, acc = lax.fori_loop(0, NC, chunk_body,
                    (jnp.full((R, 1), -jnp.inf, f32), jnp.zeros((R, 128), f32), jnp.zeros((R, DH), f32)))
                o = acc / jnp.sum(l, axis=-1, keepdims=True)
                return jnp.where(rowd == b, o, oh)
            oh = lax.fori_loop(0, B, batch_body, jnp.zeros((R, DH), f32))
            if wlate:
                @pl.when(h == wlate)
                def _(): late()
            return y + lax.dot_general(oh.astype(bf16), woT_v[:, pl.ds(pl.multiple_of(h * DH, DH), DH)], NT, preferred_element_type=f32)
        y = lax.fori_loop(0, H, head_body, jnp.zeros((R, D), f32))

        x1 = x + ga * y
        h2 = (_ln(x1) * (1 + cb) + sb).astype(bf16)
        h2f = h2.astype(f32)
        wr = wr_v[...].astype(f32).reshape(1, D)
        r = jnp.sum(h2f * wr, axis=-1, keepdims=True)
        wwait(wg_v, wsem.at[3]); wwait(wu_v, wsem.at[4]); wwait(wdT_v, wsem.at[5])
        g = jnp.dot(h2, wg_v[...], preferred_element_type=f32)
        u = jnp.dot(h2, wu_v[...], preferred_element_type=f32)
        a = (g * jax.nn.sigmoid(g) * u).astype(bf16)
        ym = lax.dot_general(a, wdT_v[...], NT, preferred_element_type=f32) * jax.nn.sigmoid(r)
        res = (x1 + gb * (h2f + (h2f * 0.0 + ym))).astype(bf16)
        o_v[...] = res[0:B]
        cp = pltpu.make_async_copy(o_v, o_hbm, wsem.at[9])
        cp.start(); cp.wait()

    def fn(A_x, A_k_cache, A_v_cache, A_wq, A_wo, B_x, B_w_r, B_w_gate, B_w_up, B_w_down, c, w_mod):
        hb = pl.BlockSpec(memory_space=pltpu.HBM)
        out = pl.pallas_call(kern,
            out_shape=jax.ShapeDtypeStruct((B, D), bf16),
            in_specs=[hb] * 11,
            out_specs=hb,
            scratch_shapes=[pltpu.VMEM((NBUF, T, DH), bf16), pltpu.VMEM((NBUF, T, DH), bf16),
                            pltpu.SemaphoreType.DMA((NBUF,)), pltpu.SemaphoreType.DMA((NBUF,)),
                            pltpu.VMEM((D, H*DH), bf16), pltpu.VMEM((D, H*DH), bf16),
                            pltpu.VMEM((D, F), bf16), pltpu.VMEM((D, F), bf16), pltpu.VMEM((D, F), bf16),
                            pltpu.VMEM((D, 6*D), bf16), pltpu.VMEM((B, D), bf16), pltpu.VMEM((B, D), bf16),
                            pltpu.VMEM((D,), bf16), pltpu.VMEM((B, D), bf16), pltpu.SemaphoreType.DMA((10,)),
                            pltpu.VMEM((H, R, DH), bf16)],
            compiler_params=pltpu.CompilerParams(vmem_limit_bytes=100*1024*1024),
        )(A_x.reshape(B, D), A_k_cache, A_v_cache, A_wq, A_wo.T, B_w_r, B_w_gate, B_w_up, B_w_down.T, c, w_mod)
        return out.reshape(B, 1, D)
    return fn


_fn = make(T=1024, NBUF=4, SUB=80, WSUB=8)


@jax.jit
def pallas_adaLN_cond__mha_block_cached__moe_arch_mod__decode_kernel(
    A_x, A_k_cache, A_v_cache, A_wq, A_wo, B_x, B_w_r, B_w_gate, B_w_up, B_w_down, c, w_mod
):
    return _fn(A_x, A_k_cache, A_v_cache, A_wq, A_wo, B_x, B_w_r, B_w_gate, B_w_up, B_w_down, c, w_mod)
```
